```python
import os as _os
_os.environ.setdefault("JAX_PLATFORMS", "cpu")
import jax
import jax.numpy as jnp

def _softmax(x, axis=-1):
    return jax.nn.softmax(x, axis=axis)
def _gelu(x):
    return jax.nn.gelu(x, approximate=True)
def _silu(x):
    return jax.nn.silu(x)
def _sigmoid(x):
    return jax.nn.sigmoid(x)
def _layernorm(x, axis=-1, eps=1e-5):
    m = jnp.mean(x, axis=axis, keepdims=True)
    v = jnp.var(x, axis=axis, keepdims=True)
    return (x - m) / jnp.sqrt(v + eps)
def _scatter_add(tgt, idx, src, axis=0):
    return tgt.at[idx].add(src)
def _segment_sum(src, seg, n):
    return jax.ops.segment_sum(src, seg, n)
class _Rng:
    def __init__(self, key):
        self._k = key
    def _next(self):
        self._k, sub = jax.random.split(self._k)
        return sub
    def normal(self, shape):
        return jax.random.normal(self._next(), shape, dtype=jnp.bfloat16)
    def randint(self, lo, hi, shape):
        return jax.random.randint(self._next(), shape, lo, hi, dtype=jnp.int32)
    def uniform(self, shape, lo=0.0, hi=1.0):
        return jax.random.uniform(self._next(), shape, jnp.bfloat16, lo, hi)
    def permutation(self, n):
        return jax.random.permutation(self._next(), n)


kernel_name = 'concat_heads__sliding_local_dilated__sliding_block__prompt'

def setup_inputs():
    _rng = _Rng(jax.random.key(int.from_bytes(__import__("os").urandom(4), "little")))
    _w = (lambda a: (lambda t: t.astype(jnp.bfloat16) if jnp.issubdtype(t.dtype, jnp.floating) else t)(jnp.asarray(a)))
    def _A_setup():
        B, S, D = 1, 2048, 1024
        return {
            "x": _w((lambda *s: _rng.normal(s) * 0.2)(B, S, D)),
            "wqkv": _w((lambda *s: _rng.normal(s) * 0.2)(D, 3 * D)),
            "wo": _w((lambda *s: _rng.normal(s) * 0.05)(D, D)),
        }
    _A_in = _A_setup()

    def _B_setup():
        B, S, D = 1, 2048, 1024
        return {
            "x": _w((lambda *s: _rng.normal(s) * 0.2)(B, S, D)),
            "wqkv": _w((lambda *s: _rng.normal(s) * 0.2)(D, 3 * D)),
            "wo": _w((lambda *s: _rng.normal(s) * 0.05)(D, D)),
        }
    _B_in = _B_setup()

    return {
        "A_x": _A_in["x"],
        "A_wqkv": _A_in["wqkv"],
        "A_wo": _A_in["wo"],
        "B_x": _B_in["x"],
        "B_wqkv": _B_in["wqkv"],
        "B_wo": _B_in["wo"],
    }

def reference(A_x, A_wqkv, A_wo, B_x, B_wqkv, B_wo):
    def _A_ref(x, wqkv, wo):
        B, S, D = x.shape
        H = 32; Dh = D // H
        W, dil = 8, 2
        qkv = (lambda x, *d: x.transpose(*d))((x @ wqkv).reshape(B, S, 3, H, Dh), 2, 0, 3, 1, 4)
        q, k, v = qkv[0], qkv[1], qkv[2]
        scale = Dh ** -0.5
        pos = jnp.arange(S)
        off = jnp.arange(W) * dil
        idx = pos[:, None] - off[None, :]
        mask = idx >= 0
        idx_c = jnp.where(mask, idx, 0).reshape(-1)
        kg = k[:, :, idx_c, :].reshape(B, H, S, W, Dh)
        vg = v[:, :, idx_c, :].reshape(B, H, S, W, Dh)
        logits = jnp.einsum("bhsd,bhswd->bhsw", q, kg) * scale
        logits = jnp.where(mask[None, None, :, :], logits, -1e9)
        attn = _softmax(logits, axis=-1)
        o = jnp.einsum("bhsw,bhswd->bhsd", attn, vg)
        return (lambda x, *d: x.transpose(*d))(o, 0, 2, 1, 3).reshape(B, S, D) @ wo

    def _B_ref(x, wqkv, wo):
        B, S, D = x.shape
        H = 32; Dh = D // H; W = 256
        qkv = (lambda x, *d: x.transpose(*d))((x @ wqkv).reshape(B, S, 3, H, Dh), 2, 0, 3, 1, 4)
        q, k, v = qkv[0], qkv[1], qkv[2]
        scores = jnp.einsum("bhqd,bhkd->bhqk", q, k) * (Dh ** -0.5)
        idx = jnp.arange(S)
        mask = (idx[:, None] - idx[None, :] >= 0) & (idx[:, None] - idx[None, :] < W)
        scores = jnp.where(mask[None, None], scores, -1e9)
        p = _softmax(scores, axis=-1)
        o = jnp.einsum("bhqk,bhkd->bhqd", p, v)
        return (lambda x, *d: x.transpose(*d))(o, 0, 2, 1, 3).reshape(B, S, D) @ wo

    a = _A_ref(A_x, A_wqkv, A_wo)
    b = _B_ref(B_x, B_wqkv, B_wo)
    return jnp.concatenate([a, b], axis=-1)
```

```python
import functools

import jax
import jax.numpy as jnp
from jax import lax
import jax.experimental.pallas as pl
import jax.experimental.pallas.tpu as pltpu

S = 2048
D = 1024
H = 32
DH = 32
WIN_B = 256
WIN_A = 8
DIL_A = 2
T = 256
QB = 128
KB = QB + WIN_B
NEG = -1e9


def _kernel(xa_ref, wqkva_ref, woa_ref, xb_ref, wqkvb_ref, wob_ref, o_ref,
            ka_buf, va_buf, kb_scr, vb_scr, ob_scr):
    i = pl.program_id(0)
    scale = DH ** -0.5
    f32 = jnp.float32
    bf16 = jnp.bfloat16

    @pl.when(i == 0)
    def _():
        ka_buf[0:16, :] = jnp.zeros((16, D), f32)
        va_buf[0:16, :] = jnp.zeros((16, D), f32)
        kb_scr[0:WIN_B, :] = jnp.zeros((WIN_B, D), bf16)
        vb_scr[0:WIN_B, :] = jnp.zeros((WIN_B, D), bf16)

    qkv = jnp.dot(xa_ref[...], wqkva_ref[...], preferred_element_type=f32)
    qa = qkv[:, :D].astype(bf16).astype(f32) * scale
    ka_buf[16:16 + T, :] = qkv[:, D:2 * D].astype(bf16).astype(f32)
    va_buf[16:16 + T, :] = qkv[:, 2 * D:].astype(bf16).astype(f32)

    rr = lax.broadcasted_iota(jnp.int32, (128, 128), 0) // DH
    cc = lax.broadcasted_iota(jnp.int32, (128, 128), 1) // DH
    bd = jnp.where(rr == cc, 1.0, 0.0).astype(bf16)
    pos = i * T + lax.broadcasted_iota(jnp.int32, (T, 128), 0)

    oa_parts = []
    for g in range(D // 128):
        sl = slice(g * 128, (g + 1) * 128)
        qg = qa[:, sl]
        logits = []
        for w in range(WIN_A):
            kw = ka_buf[16 - DIL_A * w:16 - DIL_A * w + T, sl]
            lg = jnp.dot((qg * kw).astype(bf16), bd, preferred_element_type=f32)
            logits.append(jnp.where(pos >= DIL_A * w, lg, NEG))
        m = functools.reduce(jnp.maximum, logits)
        ps = [jnp.exp(l - m) for l in logits]
        den = functools.reduce(lambda a, b: a + b, ps)
        acc = None
        for w in range(WIN_A):
            vw = va_buf[16 - DIL_A * w:16 - DIL_A * w + T, sl]
            t = ps[w] * vw
            acc = t if acc is None else acc + t
        oa_parts.append((acc / den).astype(bf16))
    oa = jnp.concatenate(oa_parts, axis=1)
    o_ref[:, :D] = jnp.dot(oa, woa_ref[...], preferred_element_type=f32).astype(o_ref.dtype)
    ka_buf[0:16, :] = ka_buf[T:T + 16, :]
    va_buf[0:16, :] = va_buf[T:T + 16, :]

    qkv = jnp.dot(xb_ref[...], wqkvb_ref[...], preferred_element_type=f32)
    qb = (qkv[:, :D] * scale).astype(bf16)
    row0 = pl.multiple_of(i * T, T)
    kb_scr[pl.ds(WIN_B + row0, T), :] = qkv[:, D:2 * D].astype(bf16)
    vb_scr[pl.ds(WIN_B + row0, T), :] = qkv[:, 2 * D:].astype(bf16)

    lane_h = lax.broadcasted_iota(jnp.int32, (QB, 128), 1) // DH
    r4 = lax.broadcasted_iota(jnp.int32, (4 * QB, KB), 0) % QB
    c4 = lax.broadcasted_iota(jnp.int32, (4 * QB, KB), 1)
    for sb in range(T // QB):
        r0 = pl.multiple_of(i * T + sb * QB, QB)
        valid = (c4 > jnp.maximum(r4, WIN_B - 1 - r0)) & (c4 <= r4 + WIN_B)
        for g in range(D // 128):
            sl = slice(g * 128, (g + 1) * 128)
            qg = qb[sb * QB:(sb + 1) * QB, sl]
            q4 = jnp.concatenate(
                [jnp.where(lane_h == j, qg, jnp.zeros_like(qg)) for j in range(4)], axis=0)
            kg = kb_scr[pl.ds(r0, KB), sl]
            vg = vb_scr[pl.ds(r0, KB), sl]
            s = lax.dot_general(q4, kg, (((1,), (1,)), ((), ())), preferred_element_type=f32)
            s = jnp.where(valid, s, NEG)
            m = jnp.max(s, axis=1, keepdims=True)
            p = jnp.exp(s - m)
            l = jnp.sum(p, axis=1, keepdims=True)
            o4 = jnp.dot(p.astype(bf16), vg, preferred_element_type=f32) / l
            og = o4[0:QB]
            for j in range(1, 4):
                og = jnp.where(lane_h == j, o4[j * QB:(j + 1) * QB], og)
            ob_scr[sb * QB:(sb + 1) * QB, sl] = og.astype(bf16)
    o_ref[:, D:] = jnp.dot(ob_scr[...], wob_ref[...], preferred_element_type=f32).astype(o_ref.dtype)


@jax.jit
def pallas_concat_heads__sliding_local_dilated__sliding_block__prompt_kernel(
    A_x: jax.Array,
    A_wqkv: jax.Array,
    A_wo: jax.Array,
    B_x: jax.Array,
    B_wqkv: jax.Array,
    B_wo: jax.Array,
):
    xa = A_x.reshape(S, D)
    xb = B_x.reshape(S, D)
    const = lambda i: (0, 0)
    out = pl.pallas_call(
        _kernel,
        grid=(S // T,),
        in_specs=[
            pl.BlockSpec((T, D), lambda i: (i, 0)),
            pl.BlockSpec((D, 3 * D), const),
            pl.BlockSpec((D, D), const),
            pl.BlockSpec((T, D), lambda i: (i, 0)),
            pl.BlockSpec((D, 3 * D), const),
            pl.BlockSpec((D, D), const),
        ],
        out_specs=pl.BlockSpec((T, 2 * D), lambda i: (i, 0)),
        out_shape=jax.ShapeDtypeStruct((S, 2 * D), A_x.dtype),
        scratch_shapes=[
            pltpu.VMEM((T + 16, D), jnp.float32),
            pltpu.VMEM((T + 16, D), jnp.float32),
            pltpu.VMEM((S + WIN_B, D), jnp.bfloat16),
            pltpu.VMEM((S + WIN_B, D), jnp.bfloat16),
            pltpu.VMEM((T, D), jnp.bfloat16),
        ],
        compiler_params=pltpu.CompilerParams(
            dimension_semantics=("arbitrary",),
            vmem_limit_bytes=100 * 1024 * 1024,
        ),
    )(xa, A_wqkv, A_wo, xb, B_wqkv, B_wo)
    return out.reshape(1, S, 2 * D)
```

```python
import functools
import math

import jax
import jax.numpy as jnp
from jax import lax
import jax.experimental.pallas as pl
import jax.experimental.pallas.tpu as pltpu

S = 2048
D = 1024
H = 32
DH = 32
WIN_B = 256
WIN_A = 8
DIL_A = 2
T = 256
QB = 128
KB = QB + WIN_B
NEG = -1e9
NG = D // 128
PAD_A = 16


def _recip(x):
    r = pl.reciprocal(x, approx=True)
    return r * (2.0 - x * r)


def _kernel(xa0_ref, xa_ref, wqkva_hbm, woa_hbm, xb_ref, wqkvb_hbm, wob_hbm, o_ref,
            wqkva_ref, woa_ref, wqkvb_ref, wob_ref, sems,
            qa_buf, ka_buf, va_buf, qb_scr, kb_scr, vb_scr, oa_scr, ob_scr):
    i = pl.program_id(0)
    scale = (DH ** -0.5) * math.log2(math.e)
    f32 = jnp.float32
    bf16 = jnp.bfloat16

    CA = 512
    NCA = 3 * D // CA

    def w_copy(n):
        if n < NCA:
            return pltpu.make_async_copy(wqkva_hbm.at[:, n * CA:(n + 1) * CA],
                                         wqkva_ref.at[:, n * CA:(n + 1) * CA], sems.at[n])
        src, dst = [(wqkvb_hbm, wqkvb_ref), (woa_hbm, woa_ref), (wob_hbm, wob_ref)][n - NCA]
        return pltpu.make_async_copy(src, dst, sems.at[n])

    NSTEP = S // T
    cur = i % 2
    nxt = 1 - cur
    row0 = pl.multiple_of(i * T, T)

    def phase1(x_ref, slot, first):
        cw = CA if first else D
        for n in range(3 * D // cw):
            if first:
                w_copy(n).wait()
            c, part = divmod(n * cw, D)
            cs = slice(part, part + cw)
            r = jnp.dot(x_ref[...], wqkva_ref[:, n * cw:(n + 1) * cw], preferred_element_type=f32)
            r = r.astype(bf16).astype(f32)
            if c == 0:
                qa_buf[slot, :, cs] = r * scale
            else:
                buf = ka_buf if c == 1 else va_buf
                for sft in range(4):
                    buf[slot, sft, PAD_A + 2 * sft:PAD_A + 2 * sft + T, cs] = r

    @pl.when(i == 0)
    def _():
        for n in range(NCA + 3):
            w_copy(n).start()
        for c in range(4):
            ka_buf[0, c, 0:PAD_A + 8, :] = jnp.zeros((PAD_A + 8, D), f32)
            va_buf[0, c, 0:PAD_A + 8, :] = jnp.zeros((PAD_A + 8, D), f32)
            for slot in range(2):
                ka_buf[slot, c, T + PAD_A:T + PAD_A + 8, :] = jnp.zeros((8, D), f32)
                va_buf[slot, c, T + PAD_A:T + PAD_A + 8, :] = jnp.zeros((8, D), f32)
        kb_scr[0:WIN_B, :] = jnp.zeros((WIN_B, D), bf16)
        vb_scr[0:WIN_B, :] = jnp.zeros((WIN_B, D), bf16)
        phase1(xa0_ref, 0, True)

    @pl.when(i + 1 < NSTEP)
    def _():
        for c in range(4):
            ka_buf[nxt, c, 0:PAD_A + 8, :] = ka_buf[cur, c, T:T + PAD_A + 8, :]
            va_buf[nxt, c, 0:PAD_A + 8, :] = va_buf[cur, c, T:T + PAD_A + 8, :]
        phase1(xa_ref, nxt, False)

    @pl.when(i == 0)
    def _():
        w_copy(NCA).wait()

    xb = xb_ref[...]

    rr = lax.broadcasted_iota(jnp.int32, (128, 128), 0) // DH
    cc = lax.broadcasted_iota(jnp.int32, (128, 128), 1) // DH
    bd = jnp.where(rr == cc, 1.0, 0.0).astype(bf16)
    pos16 = i * T + lax.broadcasted_iota(jnp.int32, (16, 128), 0)

    RC = 64
    NRC = T // RC

    def a_rows_c(buf, w, sl, c):
        cc_ = w % 4
        off = PAD_A + 2 * cc_ - DIL_A * w + c * RC
        return buf[cur, cc_, off:off + RC, sl]

    def a_prods(g):
        sl = slice(g * 128, (g + 1) * 128)
        out = []
        for c in range(NRC):
            qg = qa_buf[cur, c * RC:(c + 1) * RC, sl]
            out += [(qg * a_rows_c(ka_buf, w, sl, c)).astype(bf16) for w in range(WIN_A)]
        return jnp.concatenate(out, axis=0)

    prods = a_prods(0)
    for g in range(NG):
        sl = slice(g * 128, (g + 1) * 128)
        lg_all = jnp.dot(prods, bd, preferred_element_type=f32)
        r = jnp.dot(xb, wqkvb_ref[:, g * 128:(g + 1) * 128], preferred_element_type=f32)
        qb_scr[:, sl] = (r * scale).astype(bf16)
        r = jnp.dot(xb, wqkvb_ref[:, D + g * 128:D + (g + 1) * 128], preferred_element_type=f32)
        kb_scr[pl.ds(WIN_B + row0, T), sl] = r.astype(bf16)
        r = jnp.dot(xb, wqkvb_ref[:, 2 * D + g * 128:2 * D + (g + 1) * 128], preferred_element_type=f32)
        vb_scr[pl.ds(WIN_B + row0, T), sl] = r.astype(bf16)
        for c in range(NRC):
            logits = []
            for w in range(WIN_A):
                base = (c * WIN_A + w) * RC
                lg = lg_all[base:base + RC]
                if w > 0 and c == 0:
                    head = jnp.where(pos16 >= DIL_A * w, lg[0:16], NEG)
                    lg = jnp.concatenate([head, lg[16:]], axis=0)
                logits.append(lg)
            m = functools.reduce(jnp.maximum, logits)
            ps = [jnp.exp2(l - m) for l in logits]
            den = functools.reduce(lambda a, b: a + b, ps)
            acc = None
            for w in range(WIN_A):
                t = ps[w] * a_rows_c(va_buf, w, sl, c)
                acc = t if acc is None else acc + t
            oa_scr[c * RC:(c + 1) * RC, sl] = (acc * _recip(den)).astype(bf16)
        if g + 1 < NG:
            prods = a_prods(g + 1)

    @pl.when(i == 0)
    def _():
        w_copy(NCA + 1).wait()
        w_copy(NCA + 2).wait()

    oa = oa_scr[...]
    lane_h = lax.broadcasted_iota(jnp.int32, (QB, 128), 1) // DH
    r4 = lax.broadcasted_iota(jnp.int32, (4 * QB, 128), 0) % QB
    c4 = lax.broadcasted_iota(jnp.int32, (4 * QB, 128), 1)
    tri = c4 > r4
    it = 0
    for sb in range(T // QB):
        r0 = pl.multiple_of(i * T + sb * QB, QB)
        t0_ok = r0 >= 2 * QB
        t1_ok = r0 >= QB
        for g in range(NG):
            sl = slice(g * 128, (g + 1) * 128)
            if it % 2 == 0:
                n = it // 2
                o_ref[:, n * 128:(n + 1) * 128] = jnp.dot(
                    oa, woa_ref[:, n * 128:(n + 1) * 128], preferred_element_type=f32).astype(o_ref.dtype)
            it += 1
            qg = qb_scr[sb * QB:(sb + 1) * QB, sl]
            q4 = jnp.concatenate(
                [jnp.where(lane_h == j, qg, jnp.zeros_like(qg)) for j in range(4)], axis=0)
            kg = kb_scr[pl.ds(r0, KB), sl]
            vg = vb_scr[pl.ds(r0, KB), sl]
            s = lax.dot_general(q4, kg, (((1,), (1,)), ((), ())), preferred_element_type=f32)
            s0 = jnp.where(t0_ok, s[:, 0:128], NEG)
            s1 = jnp.where(t1_ok, s[:, 128:256], NEG)
            sc = jnp.where(tri, s0, s[:, 256:384])
            m = jnp.max(jnp.maximum(sc, s1), axis=1, keepdims=True)
            pc = jnp.exp2(sc - m)
            p1 = jnp.exp2(s1 - m)
            l = jnp.sum(pc + p1, axis=1, keepdims=True)
            zero = jnp.zeros_like(pc)
            p = jnp.concatenate([jnp.where(tri, pc, zero).astype(bf16), p1.astype(bf16),
                                 jnp.where(tri, zero, pc).astype(bf16)], axis=1)
            o4 = jnp.dot(p, vg, preferred_element_type=f32)
            og = o4[0:QB]
            lg = jnp.broadcast_to(l[0:QB], (QB, 128))
            for j in range(1, 4):
                og = jnp.where(lane_h == j, o4[j * QB:(j + 1) * QB], og)
                lg = jnp.where(lane_h == j, l[j * QB:(j + 1) * QB], lg)
            ob_scr[sb * QB:(sb + 1) * QB, sl] = (og * _recip(lg)).astype(bf16)
    o_ref[:, D:] = jnp.dot(ob_scr[...], wob_ref[...], preferred_element_type=f32).astype(o_ref.dtype)


@jax.jit
def pallas_concat_heads__sliding_local_dilated__sliding_block__prompt_kernel(
    A_x: jax.Array,
    A_wqkv: jax.Array,
    A_wo: jax.Array,
    B_x: jax.Array,
    B_wqkv: jax.Array,
    B_wo: jax.Array,
):
    xa = A_x.reshape(S, D)
    xb = B_x.reshape(S, D)
    out = pl.pallas_call(
        _kernel,
        grid=(S // T,),
        in_specs=[
            pl.BlockSpec((T, D), lambda i: (0, 0)),
            pl.BlockSpec((T, D), lambda i: (jnp.minimum(i + 1, S // T - 1), 0)),
            pl.BlockSpec(memory_space=pl.ANY),
            pl.BlockSpec(memory_space=pl.ANY),
            pl.BlockSpec((T, D), lambda i: (i, 0)),
            pl.BlockSpec(memory_space=pl.ANY),
            pl.BlockSpec(memory_space=pl.ANY),
        ],
        out_specs=pl.BlockSpec((T, 2 * D), lambda i: (i, 0)),
        out_shape=jax.ShapeDtypeStruct((S, 2 * D), A_x.dtype),
        scratch_shapes=[
            pltpu.VMEM((D, 3 * D), jnp.bfloat16),
            pltpu.VMEM((D, D), jnp.bfloat16),
            pltpu.VMEM((D, 3 * D), jnp.bfloat16),
            pltpu.VMEM((D, D), jnp.bfloat16),
            pltpu.SemaphoreType.DMA((3 * D // 512 + 3,)),
            pltpu.VMEM((2, T, D), jnp.float32),
            pltpu.VMEM((2, 4, T + PAD_A + 8, D), jnp.float32),
            pltpu.VMEM((2, 4, T + PAD_A + 8, D), jnp.float32),
            pltpu.VMEM((T, D), jnp.bfloat16),
            pltpu.VMEM((S + WIN_B, D), jnp.bfloat16),
            pltpu.VMEM((S + WIN_B, D), jnp.bfloat16),
            pltpu.VMEM((T, D), jnp.bfloat16),
            pltpu.VMEM((T, D), jnp.bfloat16),
        ],
        compiler_params=pltpu.CompilerParams(
            dimension_semantics=("arbitrary",),
            vmem_limit_bytes=100 * 1024 * 1024,
        ),
    )(xa, xa, A_wqkv, A_wo, xb, B_wqkv, B_wo)
    return out.reshape(1, S, 2 * D)
```
